```python
import os as _os
_os.environ.setdefault("JAX_PLATFORMS", "cpu")
import jax
import jax.numpy as jnp

def _softmax(x, axis=-1):
    return jax.nn.softmax(x, axis=axis)
def _gelu(x):
    return jax.nn.gelu(x, approximate=True)
def _silu(x):
    return jax.nn.silu(x)
def _sigmoid(x):
    return jax.nn.sigmoid(x)
def _layernorm(x, axis=-1, eps=1e-5):
    m = jnp.mean(x, axis=axis, keepdims=True)
    v = jnp.var(x, axis=axis, keepdims=True)
    return (x - m) / jnp.sqrt(v + eps)
def _scatter_add(tgt, idx, src, axis=0):
    return tgt.at[idx].add(src)
def _segment_sum(src, seg, n):
    return jax.ops.segment_sum(src, seg, n)
class _Rng:
    def __init__(self, key):
        self._k = key
    def _next(self):
        self._k, sub = jax.random.split(self._k)
        return sub
    def normal(self, shape):
        return jax.random.normal(self._next(), shape, dtype=jnp.bfloat16)
    def randint(self, lo, hi, shape):
        return jax.random.randint(self._next(), shape, lo, hi, dtype=jnp.int32)
    def uniform(self, shape, lo=0.0, hi=1.0):
        return jax.random.uniform(self._next(), shape, jnp.bfloat16, lo, hi)
    def permutation(self, n):
        return jax.random.permutation(self._next(), n)


kernel_name = 'standalone__gqa_block_cached__near_ridge'

def setup_inputs():
    _rng = _Rng(jax.random.key(int.from_bytes(__import__("os").urandom(4), "little")))
    _w = (lambda a: (lambda t: t.astype(jnp.bfloat16) if jnp.issubdtype(t.dtype, jnp.floating) else t)(jnp.asarray(a)))
    B, Sq, D = 8, 64, 512
    Hq, Hkv, Sk, Dh = 32, 8, 64, 128
    assert Hq % Hkv == 0, (Hq, Hkv)
    return {
        "x": _w((lambda *s: _rng.normal(s) * 0.8)(B, Sq, D)),
        "k_cache": _w((lambda *s: _rng.normal(s) * 0.8)(B, Hkv, Sk, Dh)),
        "v_cache": _w((lambda *s: _rng.normal(s) * 0.05)(B, Hkv, Sk, Dh)),
        "wq": _w((lambda *s: _rng.normal(s) * 0.8)(D, Hq * Dh) * (D ** -0.5)),
        "wo": _w((lambda *s: _rng.normal(s) * 0.05)(Hq * Dh, D) * ((Hq * Dh) ** -0.5)),
    }

def reference(x, k_cache, v_cache, wq, wo):
    B, Sq, D = x.shape
    Hq, Dh = 32, 128
    Hkv = k_cache.shape[1]
    rep = Hq // Hkv
    q = (lambda x, *d: x.transpose(*d))((x @ wq).reshape(B, Sq, Hq, Dh), 0, 2, 1, 3)
    k = jnp.repeat(k_cache, rep, axis=1)
    v = jnp.repeat(v_cache, rep, axis=1)
    scores = jnp.einsum("bhqd,bhkd->bhqk", q, k) * (Dh ** -0.5)
    p = _softmax(scores, axis=-1)
    o = jnp.einsum("bhqk,bhkd->bhqd", p, v)
    return (lambda x, *d: x.transpose(*d))(o, 0, 2, 1, 3).reshape(B, Sq, Hq * Dh) @ wo
```

```python
import jax
import jax.numpy as jnp
import jax.experimental.pallas as pl
import jax.experimental.pallas.tpu as pltpu

B, SQ, D = 8, 64, 512
HQ, HKV, SK, DH = 32, 8, 64, 128
REP = HQ // HKV
GW = REP * DH
SCALE = DH ** -0.5
NT = (((1,), (1,)), ((), ()))
F32 = jnp.float32
BF16 = jnp.bfloat16
HALF = B * SQ // 2
HB = B // 2


def _softmax_t(s_t):
    m = jnp.max(s_t, axis=0, keepdims=True)
    p = jnp.exp((s_t - m) * SCALE)
    l = jnp.sum(p, axis=0, keepdims=True)
    p = p / l
    return p.T.astype(BF16)


def _kernel(x_ref, k_ref, v_ref, wq_ref, wo_ref, o_ref, acc_ref):
    g = pl.program_id(0)

    @pl.when(g == 0)
    def _():
        acc_ref[...] = jnp.zeros_like(acc_ref)

    q_lo = jnp.dot(x_ref[0:HALF, :], wq_ref[...], preferred_element_type=F32).astype(BF16)

    q_hi = []
    o_lo = []
    for b in range(HB):
        qb = q_lo[b * SQ:(b + 1) * SQ, :]
        qg = jnp.concatenate([qb[:, r * DH:(r + 1) * DH] for r in range(REP)], axis=0)
        s_t = jax.lax.dot_general(k_ref[b, 0], qg, NT, preferred_element_type=F32)
        q_hi.append(jnp.dot(x_ref[HALF:, :], wq_ref[:, b * DH:(b + 1) * DH],
                            preferred_element_type=F32).astype(BF16))
        p = _softmax_t(s_t)
        o = jnp.dot(p, v_ref[b, 0], preferred_element_type=F32).astype(BF16)
        o_lo.append(jnp.concatenate([o[r * SQ:(r + 1) * SQ, :] for r in range(REP)], axis=1))
    o_lo = jnp.concatenate(o_lo, axis=0)

    o_hi = []
    for b in range(HB, B):
        i = b - HB
        qg = jnp.concatenate([q_hi[r][i * SQ:(i + 1) * SQ, :] for r in range(REP)], axis=0)
        s_t = jax.lax.dot_general(k_ref[b, 0], qg, NT, preferred_element_type=F32)
        acc_ref[0:HALF, i * DH:(i + 1) * DH] += jnp.dot(
            o_lo, wo_ref[:, i * DH:(i + 1) * DH], preferred_element_type=F32)
        p = _softmax_t(s_t)
        o = jnp.dot(p, v_ref[b, 0], preferred_element_type=F32).astype(BF16)
        o_hi.append(jnp.concatenate([o[r * SQ:(r + 1) * SQ, :] for r in range(REP)], axis=1))
    o_hi = jnp.concatenate(o_hi, axis=0)

    acc_ref[HALF:, :] += jnp.dot(o_hi, wo_ref[...], preferred_element_type=F32)

    @pl.when(g == HKV - 1)
    def _():
        o_ref[...] = acc_ref[...].astype(o_ref.dtype)


@jax.jit
def pallas_standalone__gqa_block_cached__near_ridge_kernel(
    x: jax.Array,
    k_cache: jax.Array,
    v_cache: jax.Array,
    wq: jax.Array,
    wo: jax.Array,
):
    x2 = x.reshape(B * SQ, D)
    out = pl.pallas_call(
        _kernel,
        grid=(HKV,),
        in_specs=[
            pl.BlockSpec((B * SQ, D), lambda g: (0, 0)),
            pl.BlockSpec((B, 1, SK, DH), lambda g: (0, g, 0, 0)),
            pl.BlockSpec((B, 1, SK, DH), lambda g: (0, g, 0, 0)),
            pl.BlockSpec((D, GW), lambda g: (0, g)),
            pl.BlockSpec((GW, D), lambda g: (g, 0)),
        ],
        out_specs=pl.BlockSpec((B * SQ, D), lambda g: (0, 0)),
        out_shape=jax.ShapeDtypeStruct((B * SQ, D), BF16),
        scratch_shapes=[pltpu.VMEM((B * SQ, D), F32)],
        compiler_params=pltpu.CompilerParams(dimension_semantics=("arbitrary",)),
    )(x2, k_cache, v_cache, wq, wo)
    return out.reshape(B, SQ, D)
```
